```python
import jax
import jax.numpy as jnp

def _softmax(x, axis=-1):
    return jax.nn.softmax(x, axis=axis)
def _gelu(x):
    return jax.nn.gelu(x, approximate=True)
def _silu(x):
    return jax.nn.silu(x)
def _sigmoid(x):
    return jax.nn.sigmoid(x)
def _layernorm(x, axis=-1, eps=1e-5):
    m = jnp.mean(x, axis=axis, keepdims=True)
    v = jnp.var(x, axis=axis, keepdims=True)
    return (x - m) / jnp.sqrt(v + eps)
def _scatter_add(tgt, idx, src, axis=0):
    return tgt.at[idx].add(src)
def _segment_sum(src, seg, n):
    return jax.ops.segment_sum(src, seg, n)
class _Rng:
    def __init__(self, key):
        self._k = key
    def _next(self):
        self._k, sub = jax.random.split(self._k)
        return sub
    def normal(self, shape):
        return jax.random.normal(self._next(), shape, dtype=jnp.bfloat16)
    def randint(self, lo, hi, shape):
        return jax.random.randint(self._next(), shape, lo, hi, dtype=jnp.int32)
    def uniform(self, shape, lo=0.0, hi=1.0):
        return jax.random.uniform(self._next(), shape, jnp.bfloat16, lo, hi)
    def permutation(self, n):
        return jax.random.permutation(self._next(), n)


kernel_name = 'gated_mix__sliding_block_cached__moe_arch_mod__decode'

def setup_inputs():
    _rng = _Rng(jax.random.key(int.from_bytes(__import__("os").urandom(4), "little")))
    _w = (lambda a: (lambda t: t.astype(jnp.bfloat16) if jnp.issubdtype(t.dtype, jnp.floating) else t)(jnp.asarray(a)))
    def _A_setup():
        B, Sq, D = 1, 1, 640
        Hq, Hkv, Sk, Dh = 32, 32, 32768, 192
        assert Hq % Hkv == 0, (Hq, Hkv)
        return {
            "x": _w((lambda *s: _rng.normal(s) * 0.05)(B, Sq, D)),
            "k_cache": _w((lambda *s: _rng.normal(s) * 0.05)(B, Hkv, Sk, Dh)),
            "v_cache": _w((lambda *s: _rng.normal(s) * 0.05)(B, Hkv, Sk, Dh)),
            "wq": _w((lambda *s: _rng.normal(s) * 0.05)(D, Hq * Dh) * (D ** -0.5)),
            "wo": _w((lambda *s: _rng.normal(s) * 0.05)(Hq * Dh, D) * ((Hq * Dh) ** -0.5)),
        }
    _A_in = _A_setup()

    def _B_setup():
        B, S, D, F, C = 1, 1, 640, 1536, 1
        return {
            "x": _w((lambda *s: _rng.normal(s) * 0.05)(B, S, D)),
            "w_r": _w((lambda *s: _rng.normal(s) * 0.05)(D)),
            "w_gate": _w((lambda *s: _rng.normal(s) * 0.05)(D, F)),
            "w_up": _w((lambda *s: _rng.normal(s) * 0.05)(D, F)),
            "w_down": _w((lambda *s: _rng.normal(s) * 0.05)(F, D)),
        }
    _B_in = _B_setup()

    return {
        "A_x": _A_in["x"],
        "A_k_cache": _A_in["k_cache"],
        "A_v_cache": _A_in["v_cache"],
        "A_wq": _A_in["wq"],
        "A_wo": _A_in["wo"],
        "B_x": _B_in["x"],
        "B_w_r": _B_in["w_r"],
        "B_w_gate": _B_in["w_gate"],
        "B_w_up": _B_in["w_up"],
        "B_w_down": _B_in["w_down"],
        "gate_w": _w((lambda *s: _rng.normal(s) * 0.05)(640)),
    }

def reference(A_x, A_k_cache, A_v_cache, A_wq, A_wo, B_x, B_w_r, B_w_gate, B_w_up, B_w_down, gate_w):
    def _A_ref(x, k_cache, v_cache, wq, wo):
        B, Sq, D = x.shape
        Hq, Dh = 32, 192
        Hkv, Sk = k_cache.shape[1], k_cache.shape[2]
        W = min(4096, max(256, Sk // 4))
        rep = Hq // Hkv
        q = (lambda x, *d: x.transpose(*d))((x @ wq).reshape(B, Sq, Hq, Dh), 0, 2, 1, 3)
        k = jnp.repeat(k_cache[:, :, Sk - W:, :], rep, axis=1)
        v = jnp.repeat(v_cache[:, :, Sk - W:, :], rep, axis=1)
        scores = jnp.einsum("bhqd,bhkd->bhqk", q, k) * (Dh ** -0.5)
        p = _softmax(scores, axis=-1)
        o = jnp.einsum("bhqk,bhkd->bhqd", p, v)
        return (lambda x, *d: x.transpose(*d))(o, 0, 2, 1, 3).reshape(B, Sq, Hq * Dh) @ wo

    def _B_ref(x, w_r, w_gate, w_up, w_down):
        B, S, D = x.shape
        C = 1
        r = x @ w_r
        idx = jnp.argsort(-r, axis=-1)[:, :C]
        idx_e = jnp.repeat(idx.reshape(B, C, 1), D, axis=2)
        x_sel = jnp.take_along_axis(x, idx_e, axis=1)
        g = _silu(x_sel @ w_gate)
        u = x_sel @ w_up
        y = (g * u) @ w_down
        r_sel = _sigmoid(jnp.take_along_axis(r, idx, axis=1))
        y = y * r_sel.reshape(B, C, 1)
        b_off = (jnp.arange(B) * S).reshape(B, 1)
        flat_idx = (idx + b_off).reshape(B * C)
        zero = (x * 0.0).reshape(B * S, D)
        upd = _scatter_add(zero, flat_idx, y.reshape(B * C, D), axis=0)
        return x + upd.reshape(B, S, D)

    x = A_x
    g = _sigmoid((x * gate_w).sum(-1, keepdims=True))
    a = _A_ref(x, A_k_cache, A_v_cache, A_wq, A_wo)
    b = _B_ref(x, B_w_r, B_w_gate, B_w_up, B_w_down)
    return g * a + (1 - g) * b
```

```python
import jax
import jax.numpy as jnp
from jax import lax
from jax.experimental import pallas as pl
from jax.experimental.pallas import tpu as pltpu

H, DH, SK, D, F = 32, 192, 32768, 640, 1536
W = min(4096, max(256, SK // 4))
NP, PW = H // 2, 2 * DH
SCALE = float(DH ** -0.5)
RING = 3
WO_BOUNDS = tuple(range(0, 5376 + 1, 768)) + (5504, 5632, 5760, 5888, 6016, 6144)
BF16, F32 = jnp.bfloat16, jnp.float32


def _sigmoid(t):
    return 1.0 / (1.0 + jnp.exp(-t))


def _kernel(x_hbm, kt, vt, wq, wo, wr_hbm, wg, wu, wd, gw_hbm, o_ref,
            xb, wrb, gwb, kb, vb, wqb, wob, wgb, wub, wdb, qs, osc, sk, sv, sw, so):
    def k_copy(i, slot):
        return pltpu.make_async_copy(
            kt.at[pl.ds(i * PW, PW), pl.ds(SK - W, W)], kb.at[slot], sk.at[slot])

    def v_copy(i, slot):
        return pltpu.make_async_copy(
            vt.at[pl.ds(i * PW, PW), pl.ds(SK - W, W)], vb.at[slot], sv.at[slot])

    c_wq = pltpu.make_async_copy(wq, wqb, sw.at[0])
    c_x = pltpu.make_async_copy(x_hbm, xb, sw.at[1])
    c_wr = pltpu.make_async_copy(wr_hbm, wrb, sw.at[2])
    c_gw = pltpu.make_async_copy(gw_hbm, gwb, sw.at[3])
    c_wg = pltpu.make_async_copy(wg, wgb, sw.at[4])
    c_wu = pltpu.make_async_copy(wu, wub, sw.at[5])
    c_wd = pltpu.make_async_copy(wd, wdb, sw.at[6])
    n_wo = len(WO_BOUNDS) - 1
    c_wo = [
        pltpu.make_async_copy(
            wo.at[pl.ds(WO_BOUNDS[j], WO_BOUNDS[j + 1] - WO_BOUNDS[j])],
            wob.at[pl.ds(WO_BOUNDS[j], WO_BOUNDS[j + 1] - WO_BOUNDS[j])],
            so.at[j])
        for j in range(n_wo)
    ]

    c_wq.start()
    c_x.start()
    c_wr.start()
    c_gw.start()
    k_copy(0, 0).start()
    v_copy(0, 0).start()
    c_wg.start()
    c_wu.start()
    c_wd.start()
    for s in range(1, RING):
        k_copy(s, s).start()
        v_copy(s, s).start()

    c_x.wait()
    x1 = xb[...].astype(F32)
    x8 = jnp.broadcast_to(x1, (8, D)).astype(BF16)
    row = lax.broadcasted_iota(jnp.int32, (8, PW), 0)
    col = lax.broadcasted_iota(jnp.int32, (8, PW), 1)
    mask = row == (col >= DH).astype(jnp.int32)
    c_wq.wait()
    for j in range(NP):
        q = jnp.dot(x8, wqb[:, j * PW:(j + 1) * PW], preferred_element_type=F32)
        qs[j] = jnp.where(mask, q, 0.0)

    def attend(i, slot, refill):
        k_copy(i, slot).wait()
        s = jnp.dot(qs[i].astype(BF16), kb[slot], preferred_element_type=F32) * SCALE
        m = jnp.max(s, axis=1, keepdims=True)
        p = jnp.exp(s - m)
        l = jnp.sum(p, axis=1, keepdims=True)
        v_copy(i, slot).wait()
        o = lax.dot_general(p.astype(BF16), vb[slot], (((1,), (1,)), ((), ())),
                            preferred_element_type=F32)
        osc[i] = jnp.where(mask, o / l, 0.0)
        if refill:
            k_copy(i + RING, slot).start()
            v_copy(i + RING, slot).start()

    attend(0, 0, True)

    c_wr.wait()
    c_gw.wait()
    c_wg.wait()
    c_wu.wait()
    g = jnp.dot(x8, wgb[...], preferred_element_type=F32)
    u = jnp.dot(x8, wub[...], preferred_element_type=F32)
    hid = (g * _sigmoid(g) * u).astype(BF16)
    c_wd.wait()
    y = jnp.dot(hid, wdb[...], preferred_element_type=F32)[0:1]
    r = jnp.sum(x1 * wrb[...].astype(F32).reshape(1, D), axis=1, keepdims=True)
    gate = _sigmoid(jnp.sum(x1 * gwb[...].astype(F32).reshape(1, D), axis=1, keepdims=True))
    b = x1 + y * _sigmoid(r)

    n_refill = NP - RING

    def body_refill(i, c):
        attend(i, i % RING, True)
        return c

    lax.fori_loop(1, n_refill, body_refill, 0)
    for c in c_wo:
        c.start()

    def body_drain(i, c):
        attend(i, i % RING, False)
        return c

    lax.fori_loop(n_refill, NP, body_drain, 0)

    a = jnp.zeros((8, D), F32)
    for j in range(n_wo):
        c_wo[j].wait()
        r0, r1 = WO_BOUNDS[j], WO_BOUNDS[j + 1]
        while r0 < r1:
            i = r0 // PW
            c0 = r0 - i * PW
            c1 = min(PW, r1 - i * PW)
            a = a + jnp.dot(osc[i, :, c0:c1].astype(BF16), wob[r0:r0 + (c1 - c0), :],
                            preferred_element_type=F32)
            r0 += c1 - c0
    a1 = jnp.sum(a, axis=0, keepdims=True)
    o_ref[...] = (gate * a1 + (1.0 - gate) * b).astype(BF16)


@jax.jit
def pallas_gated_mix__sliding_block_cached__moe_arch_mod__decode_kernel(
    A_x: jax.Array,
    A_k_cache: jax.Array,
    A_v_cache: jax.Array,
    A_wq: jax.Array,
    A_wo: jax.Array,
    B_x: jax.Array,
    B_w_r: jax.Array,
    B_w_gate: jax.Array,
    B_w_up: jax.Array,
    B_w_down: jax.Array,
    gate_w: jax.Array,
):
    del B_x
    kt = jnp.swapaxes(A_k_cache, 2, 3).reshape(H * DH, SK)
    vt = jnp.swapaxes(A_v_cache, 2, 3).reshape(H * DH, SK)
    hbm = pl.BlockSpec(memory_space=pl.ANY)
    out = pl.pallas_call(
        _kernel,
        in_specs=[hbm] * 10,
        out_specs=pl.BlockSpec(memory_space=pltpu.VMEM),
        out_shape=jax.ShapeDtypeStruct((1, D), BF16),
        scratch_shapes=[
            pltpu.VMEM((1, D), BF16),
            pltpu.VMEM((D,), BF16),
            pltpu.VMEM((D,), BF16),
            pltpu.VMEM((RING, PW, W), BF16),
            pltpu.VMEM((RING, PW, W), BF16),
            pltpu.VMEM((D, H * DH), BF16),
            pltpu.VMEM((H * DH, D), BF16),
            pltpu.VMEM((D, F), BF16),
            pltpu.VMEM((D, F), BF16),
            pltpu.VMEM((F, D), BF16),
            pltpu.VMEM((NP, 8, PW), F32),
            pltpu.VMEM((NP, 8, PW), F32),
            pltpu.SemaphoreType.DMA((RING,)),
            pltpu.SemaphoreType.DMA((RING,)),
            pltpu.SemaphoreType.DMA((7,)),
            pltpu.SemaphoreType.DMA((len(WO_BOUNDS) - 1,)),
        ],
        compiler_params=pltpu.CompilerParams(vmem_limit_bytes=64 * 1024 * 1024),
    )(A_x.reshape(1, D), kt, vt, A_wq, A_wo, B_w_r, B_w_gate, B_w_up, B_w_down, gate_w)
    return out.reshape(1, 1, D)
```

```python
import jax
import jax.numpy as jnp
from jax import lax
from jax.experimental import pallas as pl
from jax.experimental.pallas import tpu as pltpu

H, DH, SK, D, F = 32, 192, 32768, 640, 1536
W = min(4096, max(256, SK // 4))
NP, PW = H // 2, 2 * DH
SCALE = float(DH ** -0.5)
BF16, F32 = jnp.bfloat16, jnp.float32

RING = 3
SEM_A, SEM_B = RING, RING + 1
N_SEM = RING + 2
WO_SIZES = (2688, 1920, 896, 384, 128, 128)
WO_VPU = 2
WO_OFFS = tuple(sum(WO_SIZES[:j]) for j in range(len(WO_SIZES) + 1))
WO_SEMS = (SEM_A, SEM_B) + tuple((NP - RING + t) % RING for t in range(RING))
assert WO_OFFS[-1] == H * DH and N_SEM <= len(WO_SIZES) <= 2 * N_SEM
assert all(s == 128 for s in WO_SIZES[len(WO_SIZES) - WO_VPU:])


def _sigmoid(t):
    return 1.0 / (1.0 + jnp.exp(-t))


def _kernel(x_hbm, kt, vt, wq, wo, wr_hbm, wg, wu, wd, gw_hbm, o_ref,
            xb, wrb, gwb, kb, vb, wqb, wob, wgb, wub, wdb, qs, osc, sem):
    def k_copy(i, slot):
        return pltpu.make_async_copy(
            kt.at[pl.ds(i * PW, PW), pl.ds(SK - W, W)], kb.at[slot], sem.at[slot])

    def v_copy(i, slot):
        return pltpu.make_async_copy(
            vt.at[pl.ds(i * PW, PW), pl.ds(SK - W, W)], vb.at[slot], sem.at[slot])

    def wo_copy(j):
        rows = pl.ds(WO_OFFS[j], WO_SIZES[j])
        return pltpu.make_async_copy(wo.at[rows], wob.at[rows], sem.at[WO_SEMS[j % N_SEM]])

    group_a = [pltpu.make_async_copy(s, d, sem.at[SEM_A])
               for s, d in ((wq, wqb), (x_hbm, xb), (wr_hbm, wrb), (gw_hbm, gwb))]
    group_b = [pltpu.make_async_copy(s, d, sem.at[SEM_B])
               for s, d in ((wg, wgb), (wu, wub), (wd, wdb))]

    for c in group_a:
        c.start()
    k_copy(0, 0).start()
    v_copy(0, 0).start()
    for c in group_b:
        c.start()
    for s in range(1, RING):
        k_copy(s, s).start()
        v_copy(s, s).start()

    for c in group_a:
        c.wait()
    x1 = xb[...].astype(F32)
    x8 = jnp.broadcast_to(x1, (8, D)).astype(BF16)
    row = lax.broadcasted_iota(jnp.int32, (8, PW), 0)
    col = lax.broadcasted_iota(jnp.int32, (8, PW), 1)
    mask = row == (col >= DH).astype(jnp.int32)
    for j in range(NP):
        q = jnp.dot(x8, wqb[:, j * PW:(j + 1) * PW], preferred_element_type=F32)
        qs[j] = jnp.where(mask, q, 0.0)

    r = jnp.sum(x1 * wrb[...].astype(F32).reshape(1, D), axis=1, keepdims=True)
    gate = _sigmoid(jnp.sum(x1 * gwb[...].astype(F32).reshape(1, D), axis=1, keepdims=True))
    for c in group_b:
        c.wait()
    g = jnp.dot(x8, wgb[...], preferred_element_type=F32)
    u = jnp.dot(x8, wub[...], preferred_element_type=F32)
    hid = (g * _sigmoid(g) * u).astype(BF16)
    y = jnp.dot(hid, wdb[...], preferred_element_type=F32)[0:1]
    b_part = (1.0 - gate) * (x1 + y * _sigmoid(r))

    def attend(i, carry):
        slot = i % RING
        k_copy(i, slot).wait()
        v_copy(i, slot).wait()
        s = jnp.dot(qs[i].astype(BF16), kb[slot], preferred_element_type=F32) * SCALE
        m = jnp.max(s, axis=1, keepdims=True)
        p = jnp.exp(s - m)
        l = jnp.sum(p, axis=1, keepdims=True)
        o = lax.dot_general(p.astype(BF16), vb[slot], (((1,), (1,)), ((), ())),
                            preferred_element_type=F32)
        osc[i] = jnp.where(mask, o / l, 0.0)

        @pl.when(i + RING < NP)
        def _():
            k_copy(i + RING, slot).start()
            v_copy(i + RING, slot).start()

        @pl.when(i == NP - RING - 1)
        def _():
            wo_copy(0).start()
            wo_copy(1).start()

        for t in range(RING):
            @pl.when(i == NP - RING + t)
            def _():
                wo_copy(2 + t).start()

        return carry

    lax.fori_loop(0, NP, attend, 0)

    n_wo = len(WO_SIZES)
    o_cols = {}
    for j in range(n_wo - WO_VPU, n_wo):
        i, c0 = divmod(WO_OFFS[j], PW)
        o_flat = jnp.sum(osc[i, :, c0:c0 + 128], axis=0, keepdims=True).astype(BF16).astype(F32)
        o_cols[j] = jnp.broadcast_to(o_flat, (128, 128)).T
    a = jnp.zeros((8, D), F32)
    for j in range(n_wo):
        wo_copy(j).wait()
        if j + N_SEM < n_wo:
            wo_copy(j + N_SEM).start()
        r0, r1 = WO_OFFS[j], WO_OFFS[j + 1]
        if j >= n_wo - WO_VPU:
            wf = wob[r0:r1, :].astype(F32)
            parts = [(wf[:, t * 128:(t + 1) * 128] * o_cols[j]).reshape(16, 8, 128).sum(axis=0)
                     for t in range(D // 128)]
            a = a + jnp.concatenate(parts, axis=1)
            continue
        while r0 < r1:
            i, c0 = divmod(r0, PW)
            c1 = min(PW, r1 - i * PW)
            a = a + jnp.dot(osc[i, :, c0:c1].astype(BF16), wob[r0:r0 + (c1 - c0), :],
                            preferred_element_type=F32)
            r0 += c1 - c0
    o_ref[...] = (gate * jnp.sum(a, axis=0, keepdims=True) + b_part).astype(BF16)


@jax.jit
def pallas_gated_mix__sliding_block_cached__moe_arch_mod__decode_kernel(
    A_x: jax.Array,
    A_k_cache: jax.Array,
    A_v_cache: jax.Array,
    A_wq: jax.Array,
    A_wo: jax.Array,
    B_x: jax.Array,
    B_w_r: jax.Array,
    B_w_gate: jax.Array,
    B_w_up: jax.Array,
    B_w_down: jax.Array,
    gate_w: jax.Array,
):
    del B_x
    kt = jnp.swapaxes(A_k_cache, 2, 3).reshape(H * DH, SK)
    vt = jnp.swapaxes(A_v_cache, 2, 3).reshape(H * DH, SK)
    hbm = pl.BlockSpec(memory_space=pl.ANY)
    out = pl.pallas_call(
        _kernel,
        in_specs=[hbm] * 10,
        out_specs=pl.BlockSpec(memory_space=pltpu.VMEM),
        out_shape=jax.ShapeDtypeStruct((1, D), BF16),
        scratch_shapes=[
            pltpu.VMEM((1, D), BF16),
            pltpu.VMEM((D,), BF16),
            pltpu.VMEM((D,), BF16),
            pltpu.VMEM((RING, PW, W), BF16),
            pltpu.VMEM((RING, PW, W), BF16),
            pltpu.VMEM((D, H * DH), BF16),
            pltpu.VMEM((H * DH, D), BF16),
            pltpu.VMEM((D, F), BF16),
            pltpu.VMEM((D, F), BF16),
            pltpu.VMEM((F, D), BF16),
            pltpu.VMEM((NP, 8, PW), F32),
            pltpu.VMEM((NP, 8, PW), F32),
            pltpu.SemaphoreType.DMA((N_SEM,)),
        ],
        compiler_params=pltpu.CompilerParams(vmem_limit_bytes=64 * 1024 * 1024),
    )(A_x.reshape(1, D), kt, vt, A_wq, A_wo, B_w_r, B_w_gate, B_w_up, B_w_down, gate_w)
    return out.reshape(1, 1, D)
```
